```python
import jax
import jax.numpy as jnp

def _softmax(x, axis=-1):
    return jax.nn.softmax(x, axis=axis)
def _gelu(x):
    return jax.nn.gelu(x, approximate=True)
def _silu(x):
    return jax.nn.silu(x)
def _sigmoid(x):
    return jax.nn.sigmoid(x)
def _layernorm(x, axis=-1, eps=1e-5):
    m = jnp.mean(x, axis=axis, keepdims=True)
    v = jnp.var(x, axis=axis, keepdims=True)
    return (x - m) / jnp.sqrt(v + eps)
def _scatter_add(tgt, idx, src, axis=0):
    return tgt.at[idx].add(src)
def _segment_sum(src, seg, n):
    return jax.ops.segment_sum(src, seg, n)
class _Rng:
    def __init__(self, key):
        self._k = key
    def _next(self):
        self._k, sub = jax.random.split(self._k)
        return sub
    def normal(self, shape):
        return jax.random.normal(self._next(), shape, dtype=jnp.bfloat16)
    def randint(self, lo, hi, shape):
        return jax.random.randint(self._next(), shape, lo, hi, dtype=jnp.int32)
    def uniform(self, shape, lo=0.0, hi=1.0):
        return jax.random.uniform(self._next(), shape, jnp.bfloat16, lo, hi)
    def permutation(self, n):
        return jax.random.permutation(self._next(), n)


kernel_name = 'interleave_layers__sliding_local_dilated__spectral_gfnet__prompt'

def setup_inputs():
    _rng = _Rng(jax.random.key(int.from_bytes(__import__("os").urandom(4), "little")))
    _w = (lambda a: (lambda t: t.astype(jnp.bfloat16) if jnp.issubdtype(t.dtype, jnp.floating) else t)(jnp.asarray(a)))
    def _A_setup():
        B, S, D = 1, 2048, 1024
        return {
            "x": _w((lambda *s: _rng.normal(s) * 0.05)(B, S, D)),
            "wqkv": _w((lambda *s: _rng.normal(s) * 0.05)(D, 3 * D)),
            "wo": _w((lambda *s: _rng.normal(s) * 0.05)(D, D)),
        }
    _A_in = _A_setup()

    def _B_setup():
        B, S, D = 1, 2048, 1024
        Df = D // 2 + 1
        return {
            "x": _w((lambda *s: _rng.normal(s) * 0.05)(B, S, D)),
            "w_r": _w((lambda *s: _rng.normal(s) * 0.05)(S, Df) * 0.02),
            "w_i": _w((lambda *s: _rng.normal(s) * 0.05)(S, Df) * 0.02),
        }
    _B_in = _B_setup()

    return {
        "A_x": _A_in["x"],
        "A_wqkv": _A_in["wqkv"],
        "A_wo": _A_in["wo"],
        "B_x": _B_in["x"],
        "B_w_r": _B_in["w_r"],
        "B_w_i": _B_in["w_i"],
    }

def reference(A_x, A_wqkv, A_wo, B_x, B_w_r, B_w_i):
    def _A_ref(x, wqkv, wo):
        B, S, D = x.shape
        H = 32; Dh = D // H
        W, dil = 8, 2
        qkv = (lambda x, *d: x.transpose(*d))((x @ wqkv).reshape(B, S, 3, H, Dh), 2, 0, 3, 1, 4)
        q, k, v = qkv[0], qkv[1], qkv[2]
        scale = Dh ** -0.5
        pos = jnp.arange(S)
        off = jnp.arange(W) * dil
        idx = pos[:, None] - off[None, :]
        mask = idx >= 0
        idx_c = jnp.where(mask, idx, 0).reshape(-1)
        kg = k[:, :, idx_c, :].reshape(B, H, S, W, Dh)
        vg = v[:, :, idx_c, :].reshape(B, H, S, W, Dh)
        logits = jnp.einsum("bhsd,bhswd->bhsw", q, kg) * scale
        logits = jnp.where(mask[None, None, :, :], logits, -1e9)
        attn = _softmax(logits, axis=-1)
        o = jnp.einsum("bhsw,bhswd->bhsd", attn, vg)
        return (lambda x, *d: x.transpose(*d))(o, 0, 2, 1, 3).reshape(B, S, D) @ wo

    def _B_ref(x, w_r, w_i):
        B, S, D = x.shape
        X = (lambda x, axes=(-2,-1): jnp.fft.rfft2(x.astype(jnp.float32), axes=axes))(x, axes=(-2, -1))
        W = w_r + 1j * w_i
        X = X * W
        y = (lambda x, s, axes=(-2,-1): jnp.fft.irfft2(x, s=s, axes=axes).astype(jnp.bfloat16))(X, (S, D), axes=(-2, -1))
        return y

    x = A_x
    x = x + _A_ref(_layernorm(x, axis=-1), A_wqkv, A_wo)
    x = x + _B_ref(_layernorm(x, axis=-1), B_w_r, B_w_i)
    x = x + _A_ref(_layernorm(x, axis=-1), A_wqkv, A_wo)
    x = x + _B_ref(_layernorm(x, axis=-1), B_w_r, B_w_i)
    return x
```

```python
import math

import jax
import jax.numpy as jnp
import numpy as np
import jax.experimental.pallas as pl
import jax.experimental.pallas.tpu as pltpu

S, D = 2048, 1024
NT = S // 128
R = 528
CT = 4
NC = NT // CT
F32, BF16 = jnp.float32, jnp.bfloat16


def _consts():
    k2 = np.arange(128)
    md = np.zeros((8, 256, 128), np.float64)
    for n1 in range(8):
        th = 2 * np.pi * ((k2[:, None] * (n1 + 8 * k2[None, :])) % D) / D
        md[n1, :128], md[n1, 128:] = np.cos(th), -np.sin(th)
    ms = np.zeros((16, 256, 256), np.float64)
    for k1 in range(16):
        th = 2 * np.pi * ((k2[:, None] * (k1 + 16 * k2[None, :])) % S) / S
        c, s = np.cos(th), np.sin(th)
        ms[k1] = np.block([[c, -s], [s, c]])
    f = lambda a: np.ascontiguousarray(a).astype(np.float32).astype(BF16)
    return f(md), f(md.transpose(0, 2, 1)), f(ms), f(ms.transpose(0, 2, 1))


_MD, _MDI, _MS, _MSI = _consts()


def _cadd(a, b):
    if a is None:
        return b
    if b is None:
        return a
    return (a[0] + b[0], a[1] + b[1])


def _bfly(e, o, k, n, sign, want_minus):
    if o is None:
        return e, e
    if k == 0:
        t = o
    elif 4 * k == n:
        if e is None:
            raise NotImplementedError
        p = (e[0] - o[1], e[1] + o[0])
        m = (e[0] + o[1], e[1] - o[0])
        return (p, m) if sign > 0 else (m, p)
    else:
        c, s = math.cos(2 * math.pi * k / n), sign * math.sin(2 * math.pi * k / n)
        if 8 * k == n or 8 * k == 3 * n:
            r = abs(c)
            a, b = o[0] + o[1], o[0] - o[1]
            if c > 0 and s > 0:
                t = (b * r, a * r)
            elif c > 0:
                t = (a * r, b * -r)
            elif s > 0:
                t = (a * -r, b * r)
            else:
                t = (b * -r, a * -r)
        else:
            t = (o[0] * c - o[1] * s, o[0] * s + o[1] * c)
    return _cadd(e, t), ((e[0] - t[0], e[1] - t[1]) if want_minus else None)


def _fft(x, sign, nout=None):
    n = len(x)
    if n == 1:
        return x
    nout = n if nout is None else nout
    e, o = _fft(x[0::2], sign), _fft(x[1::2], sign)
    out = [None] * n
    for k in range(n // 2):
        out[k], out[k + n // 2] = _bfly(e[k], o[k], k, n, sign, k + n // 2 < nout)
    return out[:nout]


def _dot(a, b):
    return jnp.dot(a, b, preferred_element_type=F32)


def _loop(*a, **k):
    def deco(f):
        with jax.named_scope("loop_%d_%d" % a):
            pl.loop(*a, **k)(f)
    return deco


def _spread(ref, v, n):
    for i in range(v.shape[0] // n):
        ref[pl.ds(i * (n + 1), n), :] = v[i * n:(i + 1) * n]


def _gather(ref, rows, n):
    return jnp.concatenate([ref[pl.ds(i * (n + 1), n), :] for i in range(rows // n)], axis=0)


def _unpack(u):
    return (pltpu.bitcast(u << 16, F32), pltpu.bitcast(u & jnp.uint32(0xFFFF0000), F32))


def _kernel(x_hbm, wqkv_hbm, wo_hbm, wr_hbm, wi_hbm, md_hbm, mdi_hbm, ms_hbm, msi_hbm,
            out_hbm,
            xio, wq_in, wo_in, wr_in, wi_in, md, mdi, ms, msi,
            wqt, wot, wf, xs, hb, q_s, k_s, v_s, o_s, cb, ab, hf2, zb2, ub2, tmp, tmp2, wtmp,
            sems):
    srcs = (x_hbm, wo_hbm, wr_hbm, wi_hbm, md_hbm, mdi_hbm, ms_hbm, msi_hbm)
    dsts = (xio, wo_in, wr_in, wi_in, md, mdi, ms, msi)
    cps = [pltpu.make_async_copy(s, d, sems.at[i]) for i, (s, d) in enumerate(zip(srcs, dsts))]
    wcp = [pltpu.make_async_copy(wqkv_hbm.at[:, pl.ds(p * 1024, 1024)], wq_in.at[p],
                                 sems.at[8 + p]) for p in range(3)]
    cps[0].start()
    for c in wcp:
        c.start()
    for c in cps[1:]:
        c.start()

    def ln(x):
        m = jnp.mean(x, axis=0, keepdims=True)
        xc = x - m
        v = jnp.mean(xc * xc, axis=0, keepdims=True)
        return xc * jax.lax.rsqrt(v + 1e-5)

    cps[0].wait()

    @_loop(0, NT, unroll=2)
    def _(t):
        x = xio[pl.ds(pl.multiple_of(t * 128, 128), 128), :].astype(F32).T
        xs[t] = x
        hb[t] = ln(x).astype(BF16)

    for p in range(3):
        wcp[p].wait()

        @_loop(0, 4)
        def _(g):
            for ct in range(8):
                w = wq_in[p, pl.ds(ct * 128, 128), pl.ds(pl.multiple_of(g * 256, 256), 256)]
                tmp[ct, pl.ds(0, 256), :] = w.astype(F32).T
                for h in range(8):
                    for e in range(2):
                        tmp2[ct, pl.ds(h * 2 + e, 16, stride=17), :] = (
                            tmp[ct, pl.ds(h * 32 + e, 16, stride=2), :])
                wqt[g, pl.ds(p * 256, 256), pl.ds(ct * 128, 128)] = _gather(tmp2.at[ct], 256, 16).astype(BF16)

    zpad = jnp.zeros((D, 128), BF16)
    k_s[0] = zpad
    v_s[0] = zpad
    lane = jax.lax.broadcasted_iota(jnp.int32, (8, 128), 1)

    def qkv(t):
        g, c = t // NC, t % NC
        rhs = jnp.concatenate([hb[c * CT + i] for i in range(CT)], axis=1)
        r0 = pl.multiple_of(g * 256, 256)
        for p, (dst, off) in enumerate(((q_s, 0), (k_s, 1), (v_s, 1))):
            y = _dot(wqt[g, pl.ds(p * 256, 256), :], rhs).astype(BF16)
            for i in range(CT):
                dst[c * CT + i + off, pl.ds(r0, 256), :] = y[:, i * 128:(i + 1) * 128]

    def shifted(ref, tile, r):
        cur = pltpu.bitcast(ref[tile + 1, pl.ds(r, 16), :], jnp.uint32)
        prv = pltpu.bitcast(ref[tile, pl.ds(r, 16), :], jnp.uint32)
        out = [cur]
        for j in range(1, 8):
            out.append(pltpu.roll(jnp.where(lane >= 128 - 2 * j, prv, cur), 2 * j, 1))
        return out

    def attn(t):
        g, c = t // NC, t % NC
        for i in range(CT):
            tile = c * CT + i
            lg = [None] * 8
            for dp in range(16):
                r = pl.multiple_of(g * 256 + dp * 16, 16)
                ql, qh = _unpack(pltpu.bitcast(q_s[tile, pl.ds(r, 16), :], jnp.uint32))
                for j, u in enumerate(shifted(k_s, tile, r)):
                    kl, kh = _unpack(u)
                    pr = ql * kl + qh * kh
                    lg[j] = pr if lg[j] is None else lg[j] + pr
            pos = lane + tile * 128
            lg = [l * (32 ** -0.5) for l in lg]
            lg = [lg[0]] + [jnp.where(pos >= 2 * j, lg[j], -1e9) for j in range(1, 8)]
            m = lg[0]
            for l in lg[1:]:
                m = jnp.maximum(m, l)
            ex = [jnp.exp(l - m) for l in lg]
            inv = 1.0 / sum(ex[1:], ex[0])
            a = [e * inv for e in ex]
            for dp in range(16):
                r = pl.multiple_of(g * 256 + dp * 16, 16)
                ol = oh = None
                for j, u in enumerate(shifted(v_s, tile, r)):
                    vl, vh = _unpack(u)
                    ol = a[j] * vl if ol is None else ol + a[j] * vl
                    oh = a[j] * vh if oh is None else oh + a[j] * vh
                o_s[tile, pl.ds(r, 16), :] = jnp.concatenate([ol, oh], axis=0).astype(BF16)

    def prep_rest():
        for c in cps[1:]:
            c.wait()

        @_loop(0, 4)
        def _(g):
            for ct in range(8):
                v = wo_in[pl.ds(pl.multiple_of(g * 256, 256), 256),
                                pl.ds(ct * 128, 128)].astype(F32)
                _spread(tmp.at[ct], v, 32)
                v = jnp.concatenate([tmp[ct, pl.ds(d, 8, stride=33), :] for d in range(32)], axis=0)
                wot[pl.ds(ct * 128, 128), pl.ds(pl.multiple_of(g * 256, 256), 256)] = v.T.astype(BF16)

        row = jax.lax.broadcasted_iota(jnp.int32, (128, 128), 0)
        col = jax.lax.broadcasted_iota(jnp.int32, (128, S), 0)
        for part, src in enumerate((wr_in, wi_in)):
            for ct in range(5):
                if ct < 4:
                    _spread(wtmp, src[pl.ds(ct * 128, 128), :].astype(F32).T, 16)
                else:
                    _spread(wtmp, jnp.where(col == 0, src[pl.ds(512, 1), :].astype(F32), 0.0).T, 16)
                sc = 2.0 / (S * D)

                @_loop(0, 16, unroll=4)
                def _(k1):
                    w = wtmp[pl.ds(k1, 128, stride=17), :].T * sc
                    if ct in (0, 4):
                        w = jnp.where(row == 0, w * 0.5, w)
                    n = 128 if ct < 4 else 16
                    wf[k1, pl.ds(ct * 128, n), pl.ds(part * 128, 128)] = w[:n].astype(BF16)

    def layer(first):
        qkv(0)

        @_loop(1, 4 * NC)
        def _(t):
            attn(t - 1)
            qkv(t)

        if first:
            prep_rest()
        attn(4 * NC - 1)

        for c in range(NC):
            hf, zb, ub = hf2.at[c % 2], zb2.at[c % 2], ub2.at[c % 2]
            y = _dot(wot[...], jnp.concatenate([o_s[c * CT + i] for i in range(CT)], axis=1))
            for i in range(CT):
                x = xs[c * CT + i] + y[:, i * 128:(i + 1) * 128]
                xs[c * CT + i] = x
                _spread(hf.at[i], ln(x), 8)
            for n1 in range(8):
                rhs = jnp.concatenate(
                    [hf[i, pl.ds(n1, 128, stride=9), :].astype(BF16) for i in range(CT)], axis=1)
                zb[n1] = _dot(md[n1], rhs)
            for i in range(CT):
                for rb in range(16):
                    z = [(zb[n1, pl.ds(rb * 8, 8), pl.ds(i * 128, 128)],
                          zb[n1, pl.ds(128 + rb * 8, 8), pl.ds(i * 128, 128)]) for n1 in range(8)]
                    for k1, v in enumerate(_fft(z, -1, 5 if rb < 2 else 4)):
                        cb[c * CT + i, pl.ds(k1 * 128 + rb * 8, 8), pl.ds(0, 128)] = v[0]
                        cb[c * CT + i, pl.ds(k1 * 128 + rb * 8, 8), pl.ds(128, 128)] = v[1]

        @_loop(0, R // 16)
        def _(rb):
            res = []
            for hlf in range(2):
                r = pl.ds(pl.multiple_of(rb * 16 + hlf * 8, 8), 8)
                res.append(_fft([(cb[n, r, pl.ds(0, 128)], cb[n, r, pl.ds(128, 128)])
                                 for n in range(16)], -1))
            r = pl.ds(pl.multiple_of(rb * 16, 16), 16)
            for k1 in range(16):
                for p in range(2):
                    ab[k1, r, pl.ds(p * 128, 128)] = jnp.concatenate(
                        [res[0][k1][p], res[1][k1][p]], axis=0).astype(BF16)

        @_loop(0, 16, step=2)
        def _(k0):
            for k1 in (k0, k0 + 1):
                f = _dot(ab[k1], ms[k1])
                w = wf[k1].astype(F32)
                fr, fi, wr, wi = f[:, :128], f[:, 128:], w[:, :128], w[:, 128:]
                g = jnp.concatenate([fr * wr - fi * wi, fr * wi + fi * wr], axis=1)
                cb[k1] = _dot(g.astype(BF16), msi[k1])

        @_loop(0, R // 8)
        def _(rb):
            r = pl.ds(pl.multiple_of(rb * 8, 8), 8)
            res = _fft([(cb[n, r, pl.ds(0, 128)], cb[n, r, pl.ds(128, 128)])
                        for n in range(16)], 1)
            for n in range(16):
                cb[n, r, pl.ds(0, 128)] = res[n][0]
                cb[n, r, pl.ds(128, 128)] = res[n][1]

        for c in range(NC):
            hf, zb, ub = hf2.at[c % 2], zb2.at[c % 2], ub2.at[c % 2]
            for i in range(CT):
                t = c * CT + i
                for rb in range(8):
                    res = []
                    for hlf in range(2):
                        r0 = rb * 16 + hlf * 8
                        z = [(cb[t, pl.ds(k1 * 128 + r0, 8), pl.ds(0, 128)],
                              cb[t, pl.ds(k1 * 128 + r0, 8), pl.ds(128, 128)])
                             if k1 < (5 if r0 == 0 else 4) else None for k1 in range(8)]
                        res.append(_fft(z, 1))
                    for n1 in range(8):
                        for p in range(2):
                            ub[n1, pl.ds(p * 128 + rb * 16, 16), pl.ds(i * 128, 128)] = (
                                jnp.concatenate([res[0][n1][p], res[1][n1][p]], axis=0).astype(BF16))
            for n1 in range(8):
                y = _dot(mdi[n1], ub[n1])
                for i in range(CT):
                    hf[i, pl.ds(n1, 128, stride=9), :] = y[:, i * 128:(i + 1) * 128]
            for i in range(CT):
                t = c * CT + i
                x = xs[t] + _gather(hf.at[i], D, 8)
                if first:
                    xs[t] = x
                    hb[t] = ln(x).astype(BF16)
                else:
                    xio[pl.ds(t * 128, 128), :] = x.T.astype(BF16)
            if not first:
                rows = pl.ds(c * CT * 128, CT * 128)
                pltpu.make_async_copy(xio.at[rows], out_hbm.at[rows], sems.at[11 + c]).start()

    layer(True)
    layer(False)
    for c in range(NC):
        rows = pl.ds(c * CT * 128, CT * 128)
        pltpu.make_async_copy(xio.at[rows], out_hbm.at[rows], sems.at[11 + c]).wait()


@jax.jit
def pallas_interleave_layers__sliding_local_dilated__spectral_gfnet__prompt_kernel(
    A_x, A_wqkv, A_wo, B_x, B_w_r, B_w_i,
):
    V = pltpu.VMEM
    L = CT * 128
    scratch = [
        V((S, D), BF16), V((3, D, D), BF16), V((D, D), BF16), V((513, S), BF16), V((513, S), BF16),
        V(_MD.shape, BF16), V(_MDI.shape, BF16), V(_MS.shape, BF16), V(_MSI.shape, BF16),
        V((4, 768, D), BF16), V((D, D), BF16), V((16, R, 256), BF16),
        V((NT, D, 128), F32), V((NT, D, 128), BF16),
        V((NT, D, 128), BF16), V((NT + 1, D, 128), BF16), V((NT + 1, D, 128), BF16),
        V((NT, D, 128), BF16),
        V((16, R, 256), F32), V((16, R, 256), BF16),
        V((2, CT, 1152, 128), F32), V((2, 8, 256, L), F32), V((2, 8, 256, L), BF16),
        V((8, 272, 128), F32), V((8, 272, 128), F32), V((2176, 128), F32),
        pltpu.SemaphoreType.DMA((11 + NC,)),
    ]
    hbm = pl.BlockSpec(memory_space=pltpu.HBM)
    out = pl.pallas_call(
        _kernel,
        in_specs=[hbm] * 9,
        out_specs=hbm,
        out_shape=jax.ShapeDtypeStruct((S, D), BF16),
        scratch_shapes=scratch,
        compiler_params=pltpu.CompilerParams(vmem_limit_bytes=120 * 1024 * 1024),
    )(A_x.reshape(S, D), A_wqkv, A_wo, B_w_r.T, B_w_i.T, _MD, _MDI, _MS, _MSI)
    return out.reshape(1, S, D)
```

```python
import math

import jax
import jax.numpy as jnp
import numpy as np
import jax.experimental.pallas as pl
import jax.experimental.pallas.tpu as pltpu

S, D = 2048, 1024
NT = S // 128
R = 528
CT = 4
NC = NT // CT
F32, BF16, U32 = jnp.float32, jnp.bfloat16, jnp.uint32


def _consts():
    k2 = np.arange(128)
    md = np.zeros((8, 256, 128), np.float64)
    for n1 in range(8):
        th = 2 * np.pi * ((k2[:, None] * (n1 + 8 * k2[None, :])) % D) / D
        md[n1, :128], md[n1, 128:] = np.cos(th), -np.sin(th)
    ms = np.zeros((16, 256, 256), np.float64)
    for k1 in range(16):
        th = 2 * np.pi * ((k2[None, :] * (k1 + 16 * k2[:, None])) % S) / S
        c, s = np.cos(th), np.sin(th)
        ms[k1] = np.block([[c, -s], [s, c]])
    f = lambda a: np.ascontiguousarray(a).astype(np.float32).astype(BF16)
    return f(md), f(md.transpose(0, 2, 1)), f(ms), f(ms.transpose(0, 2, 1) * (2.0 / (S * D)))


_MD, _MDI, _MS, _MSI = _consts()


def _cadd(a, b):
    if a is None:
        return b
    if b is None:
        return a
    return (a[0] + b[0], a[1] + b[1])


def _bfly(e, o, k, n, sign, want_minus):
    if o is None:
        return e, e
    if k == 0:
        t = o
    elif 4 * k == n:
        if e is None:
            raise NotImplementedError
        p = (e[0] - o[1], e[1] + o[0])
        m = (e[0] + o[1], e[1] - o[0])
        return (p, m) if sign > 0 else (m, p)
    else:
        c, s = math.cos(2 * math.pi * k / n), sign * math.sin(2 * math.pi * k / n)
        if 8 * k == n or 8 * k == 3 * n:
            r = abs(c)
            a, b = o[0] + o[1], o[0] - o[1]
            if c > 0 and s > 0:
                t = (b * r, a * r)
            elif c > 0:
                t = (a * r, b * -r)
            elif s > 0:
                t = (a * -r, b * r)
            else:
                t = (b * -r, a * -r)
        else:
            t = (o[0] * c - o[1] * s, o[0] * s + o[1] * c)
    return _cadd(e, t), ((e[0] - t[0], e[1] - t[1]) if want_minus else None)


def _fft(x, sign, nout=None):
    n = len(x)
    if n == 1:
        return x
    nout = n if nout is None else nout
    e, o = _fft(x[0::2], sign), _fft(x[1::2], sign)
    out = [None] * n
    for k in range(n // 2):
        out[k], out[k + n // 2] = _bfly(e[k], o[k], k, n, sign, k + n // 2 < nout)
    return out[:nout]


def _dot(a, b):
    return jnp.dot(a, b, preferred_element_type=F32)


def _loop(*a, **k):
    def deco(f):
        with jax.named_scope("loop_%d_%d" % a):
            pl.loop(*a, **k)(f)
    return deco


def _spread(ref, v, n):
    for i in range(v.shape[0] // n):
        ref[pl.ds(i * (n + 1), n), :] = v[i * n:(i + 1) * n]


def _gather(ref, rows, n):
    return jnp.concatenate([ref[pl.ds(i * (n + 1), n), :] for i in range(rows // n)], axis=0)


def _unpack(u):
    return (pltpu.bitcast(u << 16, F32), pltpu.bitcast(u & jnp.uint32(0xFFFF0000), F32))


def _mix(*gens):
    ev = sorted(((k + 0.5) / n, i) for i, (_, n) in enumerate(gens) for k in range(n))
    for _, i in ev:
        next(gens[i][0], None)
    for g, _ in gens:
        for _ in g:
            pass


def _bits16(x):
    return pltpu.bitcast(x.astype(BF16).astype(F32), U32)


def _kernel(x_hbm, wqkv_hbm, wo_hbm, wr_hbm, wi_hbm, md_hbm, mdi_hbm, ms_hbm, msi_hbm,
            out_hbm,
            xio, wq_in, wo_in, wr, wi, md, mdi, ms, msi,
            wqt, wot, xs, hb, q0, k0, v0, q1, k1_, v1, fin, o_s, cb, ab2, hf2, zb2, ub2, tmp, tmp2, tmp3, xtmp,
            sems):
    srcs = (wo_hbm, md_hbm, ms_hbm, wr_hbm, wi_hbm, msi_hbm, mdi_hbm)
    dsts = (wo_in, md, ms, wr, wi, msi, mdi)
    cps = [pltpu.make_async_copy(s, d, sems.at[i]) for i, (s, d) in enumerate(zip(srcs, dsts))]
    wcp = [[pltpu.make_async_copy(wqkv_hbm.at[:, pl.ds(p * D + g * 256, 256)], wq_in.at[g * 3 + p],
                                  sems.at[8 + g * 3 + p]) for p in range(3)] for g in range(4)]
    cols = lambda r, j: r.at[:, pl.ds(j * 256, 256)]
    xcp = [pltpu.make_async_copy(cols(x_hbm, j), xio.at[j], sems.at[20 + j]) for j in range(4)]
    rows = lambda j: pl.ds(j * 512, 512)
    ocp = [pltpu.make_async_copy(xio.at[j], cols(out_hbm, j), sems.at[24 + j]) for j in range(4)]
    for c in wcp[0] + xcp:
        c.start()

    def ln(x):
        m = jnp.mean(x, axis=0, keepdims=True)
        xc = x - m
        v = jnp.mean(xc * xc, axis=0, keepdims=True)
        return xc * jax.lax.rsqrt(v + 1e-5)

    def prep_wq(gp):
        p = gp % 3
        for ct in range(8):
            tmp[p, ct, pl.ds(0, 256), :] = wq_in[gp, pl.ds(ct * 128, 128), :].astype(F32).T
            for h in range(8):
                for e in range(2):
                    tmp2[p, ct, pl.ds(h * 2 + e, 16, stride=17), :] = (
                        tmp[p, ct, pl.ds(h * 32 + e, 16, stride=2), :])
            wqt[gp, :, pl.ds(ct * 128, 128)] = _gather(tmp2.at[p, ct], 256, 16).astype(BF16)
            yield

    def prep_wo(g):
        for ct in range(8):
            t = tmp3.at[ct]
            _spread(t, wo_in[pl.ds(g * 256, 256), pl.ds(ct * 128, 128)].astype(F32), 32)
            v = jnp.concatenate([t[pl.ds(d, 8, stride=33), :] for d in range(32)], axis=0)
            wot[pl.ds(ct * 128, 128), pl.ds(g * 256, 256)] = v.T.astype(BF16)
            yield

    for c in wcp[0]:
        c.wait()
    _loop(0, 3)(lambda p: _mix((prep_wq(p), 1)))

    for j in range(4):
        xcp[j].wait()
        if j == 3:
            for c in wcp[1] + wcp[2] + wcp[3] + cps:
                c.start()
        for hh in range(2):
            t = xtmp.at[hh]
            _spread(t, pltpu.bitcast(xio[j, :, pl.ds(hh * 128, 128)], U32), 8)
            for a in range(8):
                lo, hi = _unpack(t[pl.ds(a, 128, stride=9), :].T)
                xs[2 * a, pl.ds(j * 256 + hh * 128, 128), :] = lo
                xs[2 * a + 1, pl.ds(j * 256 + hh * 128, 128), :] = hi

    lane0 = jax.lax.broadcasted_iota(jnp.int32, (8, 128), 1) == 0
    lane0_big = jax.lax.broadcasted_iota(jnp.int32, (128, 128), 1) == 0
    row0 = jax.lax.broadcasted_iota(jnp.int32, (8, 128), 0) == 0

    bufs = ((q0, k0, v0), (q1, k1_, v1))

    def qkv(g, c):
        for i in range(CT):
            for p, dst in enumerate(bufs[g % 2]):
                u = pltpu.bitcast(_dot(wqt[g * 3 + p], hb[c * CT + i]).astype(BF16), U32)
                if p == 0:
                    dst[c * CT + i] = u
                else:
                    dst[c * CT + i + NT] = u
                    dst[c * CT + i] = jnp.where(
                        lane0_big, jnp.uint32(0), pltpu.roll(u, 1, 1))
                yield

    def attn(g, c):
        q_s, k_s, v_s = bufs[g % 2]
        for i in range(CT):
            tile = c * CT + i
            lg = [None] * 8
            for dp in range(16):
                r = pl.ds(dp * 8, 8)
                ql, qh = _unpack(q_s[tile, r, :])
                for j in range(8):
                    kl, kh = _unpack(k_s[tile + NT - 2 * j, r, :])
                    pr = ql * kl + qh * kh
                    lg[j] = pr if lg[j] is None else lg[j] + pr
                if dp % 4 == 3:
                    yield
            lg = [l * (32 ** -0.5) for l in lg]
            lg = [lg[0]] + [jnp.where(lane0 & (tile < 2 * j), -1e9, lg[j]) for j in range(1, 8)]
            m = lg[0]
            for l in lg[1:]:
                m = jnp.maximum(m, l)
            ex = [jnp.exp(l - m) for l in lg]
            inv = 1.0 / sum(ex[1:], ex[0])
            a = [e * inv for e in ex]
            for dp in range(16):
                r = pl.ds(dp * 8, 8)
                ol = oh = None
                for j in range(8):
                    vl, vh = _unpack(v_s[tile + NT - 2 * j, r, :])
                    ol = a[j] * vl if ol is None else ol + a[j] * vl
                    oh = a[j] * vh if oh is None else oh + a[j] * vh
                o_s[tile, pl.ds(g * 256 + dp * 16, 16), :] = (
                    jnp.concatenate([ol, oh], axis=0).astype(BF16))
                if dp % 4 == 3:
                    yield

    def oproj(c):
        for t in range(c * CT, c * CT + CT):
            for m in range(2):
                r = pl.ds(m * 512, 512)
                xs[t, r, :] += _dot(wot[r, :], o_s[t])
                yield

    def fwd(c):
        hf, zb, ab = hf2.at[c % 2], zb2.at[c % 2], ab2.at[c % 2]
        for i in range(CT):
            _spread(hf.at[i], ln(xs[c * CT + i]), 8)
            yield
        for n1 in range(8):
            rhs = jnp.concatenate(
                [hf[i, pl.ds(n1, 128, stride=9), :].astype(BF16) for i in range(CT)], axis=1)
            zb[n1] = _dot(md[n1], rhs)
            yield
        for i in range(CT):
            for rb in range(8):
                res = []
                for r0 in (rb * 16, rb * 16 + 8):
                    z = [(zb[n1, pl.ds(r0, 8), pl.ds(i * 128, 128)],
                          zb[n1, pl.ds(128 + r0, 8), pl.ds(i * 128, 128)]) for n1 in range(8)]
                    o = _fft(z, -1, 5 if r0 == 0 else 4)
                    if r0 == 0:
                        o[0] = tuple(jnp.where(row0, 0.5 * v, v) for v in o[0])
                        o[4] = tuple(jnp.where(row0, 0.5 * v, 0.0) for v in o[4])
                    elif r0 == 8:
                        o.append((jnp.zeros((8, 128), F32),) * 2)
                    res.append(o)
                for k1 in range(len(res[0])):
                    for p in range(2):
                        ab[i, pl.ds(k1 * 128 + rb * 16, 16), pl.ds(p * 128, 128)] = (
                            jnp.concatenate([res[0][k1][p], res[1][k1][p]], axis=0).astype(BF16))
            cb[c * CT + i] = _dot(ab[i], ms[c * CT + i])
            yield

    def filt(r, w):
        f = _fft([(cb[n, r, pl.ds(0, 128)], cb[n, r, pl.ds(128, 128)]) for n in range(16)], -1)
        g = []
        for k1 in range(16):
            a, b = w(wr, k1), w(wi, k1)
            g.append((f[k1][0] * a - f[k1][1] * b, f[k1][0] * b + f[k1][1] * a))
        for n, v in enumerate(_fft(g, 1)):
            cb[n, r, pl.ds(0, 128)] = v[0]
            cb[n, r, pl.ds(128, 128)] = v[1]

    def inv(c):
        hf, ub = hf2.at[c % 2], ub2.at[c % 2]
        for i in range(CT):
            t = c * CT + i
            cb[t] = _dot(cb[t].astype(BF16), msi[t])
            for rb in range(8):
                res = []
                for r0 in (rb * 16, rb * 16 + 8):
                    z = [(cb[t, pl.ds(k1 * 128 + r0, 8), pl.ds(0, 128)],
                          cb[t, pl.ds(k1 * 128 + r0, 8), pl.ds(128, 128)])
                         if k1 < (5 if r0 == 0 else 4) else None for k1 in range(8)]
                    res.append(_fft(z, 1))
                for n1 in range(8):
                    for p in range(2):
                        ub[n1, pl.ds(p * 128 + rb * 16, 16), pl.ds(i * 128, 128)] = (
                            jnp.concatenate([res[0][n1][p], res[1][n1][p]], axis=0).astype(BF16))
            yield
        for n1 in range(8):
            yield
            y = _dot(mdi[n1], ub[n1])
            for i in range(CT):
                hf[i, pl.ds(n1, 128, stride=9), :] = y[:, i * 128:(i + 1) * 128]
        return [xs[c * CT + i] + _gather(hf.at[i], D, 8) for i in range(CT)]

    def chain_wo():
        for g in range(4):
            yield from prep_wo(g)

    def middle(first):
        for g in range(3):
            @_loop(0, NC)
            def _(c):
                _mix((qkv(g + 1, c), 3 * CT), (attn(g, c), 8 * CT))

        if first:
            for c in cps:
                c.wait()
        for c in range(NC + 2):
            _mix(*[(f(*a, c - d), n) for d, (f, a, n) in enumerate((
                (attn, (3,), 8 * CT), (oproj, (), 2 * CT), (fwd, (), 2 * CT + 8)))
                if 0 <= c - d < NC],
                *([(g, 8) for g in [chain_wo()]] if first and c == 0 else []))

        @_loop(0, 32)
        def _(rb):
            r16 = pl.ds(pl.multiple_of(rb * 16, 16), 16)
            for hlf in range(2):
                filt(pl.ds(pl.multiple_of(rb * 16 + hlf * 8, 8), 8),
                     lambda w, k1: w[r16, pl.ds(k1 * 128, 128)].astype(F32)[hlf * 8:hlf * 8 + 8])

        filt(pl.ds(512, 8), lambda w, k1: jnp.broadcast_to(
            w[pl.ds(512, 1), pl.ds(k1 * 128, 128)].astype(F32), (8, 128)))

    def ln0(c):
        for t in range(c * CT, c * CT + CT):
            hb[t] = ln(xs[t]).astype(BF16)
            yield

    _mix((ln0(0), 1))
    for c in range(NC):
        gs = [(qkv(0, c), 3 * CT)]
        if c + 1 < NC:
            gs.append((ln0(c + 1), CT))
        if c == 1:
            for w in wcp[1] + wcp[2] + wcp[3]:
                w.wait()
        if c > 0:
            gs += [(prep_wq(c * 3 + p), 8) for p in range(3)]
        _mix(*gs)
    middle(True)

    def nxt(c):
        for i, x in enumerate((yield from inv(c))):
            xs[c * CT + i] = x
            hb[c * CT + i] = ln(x).astype(BF16)
            yield

    for c in range(NC + 1):
        _mix(*([(nxt(c), 2 * CT + 8)] if c < NC else []),
             *([(qkv(0, c - 1), 3 * CT)] if c else []))
    middle(False)
    def last(c):
        x = yield from inv(c)
        for i in range(0, CT, 2):
            u = (_bits16(x[i]) >> 16) | _bits16(x[i + 1])
            a = (c * CT + i) // 2
            for ct in range(8):
                ut = u[ct * 128:(ct + 1) * 128].T
                for qq in range(4):
                    fin[ct * 4 + qq, pl.ds(a, 32, stride=9), :] = ut[qq * 32:(qq + 1) * 32]
    for c in range(0, NC, 2):
        _mix((last(1 - 1 + c), 12), (last(c + 1), 24))
    for j in range(4):
        for hh in range(2):
            for qq in range(4):
                xio[j, rows(qq), pl.ds(hh * 128, 128)] = pltpu.bitcast(
                    _gather(fin.at[(j * 2 + hh) * 4 + qq], 256, 8), BF16)
        ocp[j].start()
    for c in ocp:
        c.wait()


@jax.jit
def pallas_interleave_layers__sliding_local_dilated__spectral_gfnet__prompt_kernel(
    A_x, A_wqkv, A_wo, B_x, B_w_r, B_w_i,
):
    V = pltpu.VMEM
    L = CT * 128
    scratch = [
        V((4, S, 256), BF16), V((12, D, 256), BF16), V((D, D), BF16),
        V((513, S), BF16), V((513, S), BF16),
        V(_MD.shape, BF16), V(_MDI.shape, BF16), V(_MS.shape, BF16), V(_MSI.shape, BF16),
        V((12, 256, D), BF16), V((D, D), BF16),
        V((NT, D, 128), F32), V((NT, D, 128), BF16),
        *([V((NT, 128, 128), U32), V((2 * NT, 128, 128), U32), V((2 * NT, 128, 128), U32)] * 2),
        V((32, 288, 128), U32),
        V((NT, D, 128), BF16),
        V((16, R, 256), F32), V((2, CT, R, 256), BF16),
        V((2, CT, 1152, 128), F32), V((2, 8, 256, L), F32), V((2, 8, 256, L), BF16),
        V((3, 8, 272, 128), F32), V((3, 8, 272, 128), F32), V((8, 272, 128), F32), V((2, 1152, 128), U32),
        pltpu.SemaphoreType.DMA((28,)),
    ]
    hbm = pl.BlockSpec(memory_space=pltpu.HBM)
    out = pl.pallas_call(
        _kernel,
        in_specs=[hbm] * 9,
        out_specs=hbm,
        out_shape=jax.ShapeDtypeStruct((S, D), BF16),
        scratch_shapes=scratch,
        compiler_params=pltpu.CompilerParams(vmem_limit_bytes=124 * 1024 * 1024),
    )(A_x.reshape(S, D), A_wqkv, A_wo, B_w_r.T, B_w_i.T, _MD, _MDI, _MS, _MSI)
    return out.reshape(1, S, D)
```

```python
import math

import jax
import jax.numpy as jnp
import numpy as np
import jax.experimental.pallas as pl
import jax.experimental.pallas.tpu as pltpu

S, D = 2048, 1024
NT = S // 128
R = 528
CT = 4
NC = NT // CT
F32, BF16, U32 = jnp.float32, jnp.bfloat16, jnp.uint32


def _consts():
    k2 = np.arange(128)
    md = np.zeros((8, 256, 128), np.float64)
    for n1 in range(8):
        th = 2 * np.pi * ((k2[:, None] * (n1 + 8 * k2[None, :])) % D) / D
        md[n1, :128], md[n1, 128:] = np.cos(th), -np.sin(th)
    ms = np.zeros((16, 256, 256), np.float64)
    for k1 in range(16):
        th = 2 * np.pi * ((k2[None, :] * (k1 + 16 * k2[:, None])) % S) / S
        c, s = np.cos(th), np.sin(th)
        ms[k1] = np.block([[c, -s], [s, c]])
    f = lambda a: np.ascontiguousarray(a).astype(np.float32).astype(BF16)
    return f(md), f(md.transpose(0, 2, 1)), f(ms), f(ms.transpose(0, 2, 1) * (2.0 / (S * D)))


_MD, _MDI, _MS, _MSI = _consts()


def _cadd(a, b):
    if a is None:
        return b
    if b is None:
        return a
    return (a[0] + b[0], a[1] + b[1])


def _bfly(e, o, k, n, sign, want_minus):
    if o is None:
        return e, e
    if k == 0:
        t = o
    elif 4 * k == n:
        if e is None:
            raise NotImplementedError
        p = (e[0] - o[1], e[1] + o[0])
        m = (e[0] + o[1], e[1] - o[0])
        return (p, m) if sign > 0 else (m, p)
    else:
        c, s = math.cos(2 * math.pi * k / n), sign * math.sin(2 * math.pi * k / n)
        if 8 * k == n or 8 * k == 3 * n:
            r = abs(c)
            a, b = o[0] + o[1], o[0] - o[1]
            if c > 0 and s > 0:
                t = (b * r, a * r)
            elif c > 0:
                t = (a * r, b * -r)
            elif s > 0:
                t = (a * -r, b * r)
            else:
                t = (b * -r, a * -r)
        else:
            t = (o[0] * c - o[1] * s, o[0] * s + o[1] * c)
    return _cadd(e, t), ((e[0] - t[0], e[1] - t[1]) if want_minus else None)


def _fft(x, sign, nout=None):
    n = len(x)
    if n == 1:
        return x
    nout = n if nout is None else nout
    e, o = _fft(x[0::2], sign), _fft(x[1::2], sign)
    out = [None] * n
    for k in range(n // 2):
        out[k], out[k + n // 2] = _bfly(e[k], o[k], k, n, sign, k + n // 2 < nout)
    return out[:nout]


def _dot(a, b):
    return jnp.dot(a, b, preferred_element_type=F32)


def _loop(*a, **k):
    def deco(f):
        with jax.named_scope("loop_%d_%d" % a):
            pl.loop(*a, **k)(f)
    return deco


def _spread(ref, v, n):
    for i in range(v.shape[0] // n):
        ref[pl.ds(i * (n + 1), n), :] = v[i * n:(i + 1) * n]


def _gather(ref, rows, n):
    return jnp.concatenate([ref[pl.ds(i * (n + 1), n), :] for i in range(rows // n)], axis=0)


def _unpack(u):
    return (pltpu.bitcast(u << 16, F32), pltpu.bitcast(u & jnp.uint32(0xFFFF0000), F32))


def _mix(*gens):
    ev = sorted(((k + 0.5) / n, i) for i, (_, n) in enumerate(gens) for k in range(n))
    for _, i in ev:
        next(gens[i][0], None)
    for g, _ in gens:
        for _ in g:
            pass


def _bits16(x):
    return pltpu.bitcast(x.astype(BF16).astype(F32), U32)


def _kernel(x_hbm, wqkv_hbm, wo_hbm, wr_hbm, wi_hbm, md_hbm, mdi_hbm, ms_hbm, msi_hbm,
            out_hbm,
            xio, wq_in, wo_in, wr, wi, md, mdi, ms, msi,
            wqt, wot, xs, hb, qkv_s, fin, o_s, cb, ab2, hf2, zb2, ub2, tmp, tmp2, tmp3, xtmp,
            sems):
    srcs = (wo_hbm, md_hbm, ms_hbm, wr_hbm, wi_hbm, msi_hbm, mdi_hbm)
    dsts = (wo_in, md, ms, wr, wi, msi, mdi)
    cps = [pltpu.make_async_copy(s, d, sems.at[i]) for i, (s, d) in enumerate(zip(srcs, dsts))]
    wcp = [[pltpu.make_async_copy(wqkv_hbm.at[:, pl.ds(p * D + g * 256, 256)], wq_in.at[g * 3 + p],
                                  sems.at[8 + g * 3 + p]) for p in range(3)] for g in range(4)]
    cols = lambda r, j: r.at[:, pl.ds(j * 256, 256)]
    xcp = [pltpu.make_async_copy(cols(x_hbm, j), xio.at[j], sems.at[20 + j]) for j in range(4)]
    rows = lambda j: pl.ds(j * 512, 512)
    ocp = [pltpu.make_async_copy(xio.at[j], cols(out_hbm, j), sems.at[24 + j]) for j in range(4)]
    for c in wcp[0] + xcp:
        c.start()

    def ln(x):
        m = jnp.mean(x, axis=0, keepdims=True)
        xc = x - m
        v = jnp.mean(xc * xc, axis=0, keepdims=True)
        return xc * jax.lax.rsqrt(v + 1e-5)

    def prep_wq(gp):
        p = gp % 3
        for ct in range(8):
            tmp[p, ct, pl.ds(0, 256), :] = wq_in[gp, pl.ds(ct * 128, 128), :].astype(F32).T
            for h in range(8):
                for e in range(2):
                    tmp2[p, ct, pl.ds(h * 2 + e, 16, stride=17), :] = (
                        tmp[p, ct, pl.ds(h * 32 + e, 16, stride=2), :])
            wqt[gp, :, pl.ds(ct * 128, 128)] = _gather(tmp2.at[p, ct], 256, 16).astype(BF16)
            yield

    def prep_wo(g):
        for ct in range(8):
            t = tmp3.at[ct]
            _spread(t, wo_in[pl.ds(g * 256, 256), pl.ds(ct * 128, 128)].astype(F32), 32)
            v = jnp.concatenate([t[pl.ds(d, 8, stride=33), :] for d in range(32)], axis=0)
            wot[pl.ds(ct * 128, 128), pl.ds(g * 256, 256)] = v.T.astype(BF16)
            yield

    for c in wcp[0]:
        c.wait()
    _loop(0, 3)(lambda p: _mix((prep_wq(p), 1)))

    for j in range(4):
        xcp[j].wait()
        if j == 3:
            for c in wcp[1] + wcp[2] + wcp[3] + cps:
                c.start()
        for hh in range(2):
            t = xtmp.at[hh]
            _spread(t, pltpu.bitcast(xio[j, :, pl.ds(hh * 128, 128)], U32), 8)
            for a in range(8):
                lo, hi = _unpack(t[pl.ds(a, 128, stride=9), :].T)
                xs[2 * a, pl.ds(j * 256 + hh * 128, 128), :] = lo
                xs[2 * a + 1, pl.ds(j * 256 + hh * 128, 128), :] = hi

    lane0 = jax.lax.broadcasted_iota(jnp.int32, (8, 128), 1) == 0
    lane0_big = jax.lax.broadcasted_iota(jnp.int32, (128, 128), 1) == 0
    row0 = jax.lax.broadcasted_iota(jnp.int32, (8, 128), 0) == 0

    def bufs(g):
        b = (g % 2) * 5 * NT
        return [qkv_s.at[pl.ds(b + o * NT, n * NT)] for o, n in ((0, 1), (1, 2), (3, 2))]

    def qkv(g, c):
        for i in range(CT):
            for p, dst in enumerate(bufs(g)):
                u = pltpu.bitcast(_dot(wqt[g * 3 + p], hb[c * CT + i]).astype(BF16), U32)
                if p == 0:
                    dst[c * CT + i] = u
                else:
                    dst[c * CT + i + NT] = u
                    dst[c * CT + i] = jnp.where(
                        lane0_big, jnp.uint32(0), pltpu.roll(u, 1, 1))
                yield

    def attn(g, c):
        q_s, k_s, v_s = bufs(g)
        for i in range(CT):
            tile = c * CT + i
            lg = [None] * 8
            for dp in range(16):
                r = pl.ds(dp * 8, 8)
                ql, qh = _unpack(q_s[tile, r, :])
                for j in range(8):
                    kl, kh = _unpack(k_s[tile + NT - 2 * j, r, :])
                    pr = ql * kl + qh * kh
                    lg[j] = pr if lg[j] is None else lg[j] + pr
                if dp % 4 == 3:
                    yield
            lg = [l * (32 ** -0.5) for l in lg]
            lg = [lg[0]] + [jnp.where(lane0 & (tile < 2 * j), -1e9, lg[j]) for j in range(1, 8)]
            m = lg[0]
            for l in lg[1:]:
                m = jnp.maximum(m, l)
            ex = [jnp.exp(l - m) for l in lg]
            inv = 1.0 / sum(ex[1:], ex[0])
            a = [e * inv for e in ex]
            for dp in range(16):
                r = pl.ds(dp * 8, 8)
                ol = oh = None
                for j in range(8):
                    vl, vh = _unpack(v_s[tile + NT - 2 * j, r, :])
                    ol = a[j] * vl if ol is None else ol + a[j] * vl
                    oh = a[j] * vh if oh is None else oh + a[j] * vh
                o_s[tile, pl.ds(pl.multiple_of(g * 256 + dp * 16, 16), 16), :] = (
                    jnp.concatenate([ol, oh], axis=0).astype(BF16))
                if dp % 4 == 3:
                    yield

    def oproj(c):
        for t in range(c * CT, c * CT + CT):
            for m in range(2):
                r = pl.ds(m * 512, 512)
                xs[t, r, :] += _dot(wot[r, :], o_s[t])
                yield

    def fwd(c):
        hf, zb, ab = hf2.at[c % 2], zb2.at[c % 2], ab2.at[c % 2]
        for i in range(CT):
            _spread(hf.at[i], ln(xs[c * CT + i]), 8)
            yield
        for n1 in range(8):
            rhs = jnp.concatenate(
                [hf[i, pl.ds(n1, 128, stride=9), :].astype(BF16) for i in range(CT)], axis=1)
            zb[n1] = _dot(md[n1], rhs)
            yield
        for i in range(CT):
            for rb in range(8):
                res = []
                for r0 in (rb * 16, rb * 16 + 8):
                    z = [(zb[n1, pl.ds(r0, 8), pl.ds(i * 128, 128)],
                          zb[n1, pl.ds(128 + r0, 8), pl.ds(i * 128, 128)]) for n1 in range(8)]
                    o = _fft(z, -1, 5 if r0 == 0 else 4)
                    if r0 == 0:
                        o[0] = tuple(jnp.where(row0, 0.5 * v, v) for v in o[0])
                        o[4] = tuple(jnp.where(row0, 0.5 * v, 0.0) for v in o[4])
                    elif r0 == 8:
                        o.append((jnp.zeros((8, 128), F32),) * 2)
                    res.append(o)
                for k1 in range(len(res[0])):
                    for p in range(2):
                        ab[i, pl.ds(k1 * 128 + rb * 16, 16), pl.ds(p * 128, 128)] = (
                            jnp.concatenate([res[0][k1][p], res[1][k1][p]], axis=0).astype(BF16))
            cb[c * CT + i] = _dot(ab[i], ms[c * CT + i])
            yield

    def filt(r, w):
        f = _fft([(cb[n, r, pl.ds(0, 128)], cb[n, r, pl.ds(128, 128)]) for n in range(16)], -1)
        g = []
        for k1 in range(16):
            a, b = w(wr, k1), w(wi, k1)
            g.append((f[k1][0] * a - f[k1][1] * b, f[k1][0] * b + f[k1][1] * a))
        for n, v in enumerate(_fft(g, 1)):
            cb[n, r, pl.ds(0, 128)] = v[0]
            cb[n, r, pl.ds(128, 128)] = v[1]

    def inv(c):
        hf, ub = hf2.at[c % 2], ub2.at[c % 2]
        for i in range(CT):
            t = c * CT + i
            cb[t] = _dot(cb[t].astype(BF16), msi[t])
            for rb in range(8):
                res = []
                for r0 in (rb * 16, rb * 16 + 8):
                    z = [(cb[t, pl.ds(k1 * 128 + r0, 8), pl.ds(0, 128)],
                          cb[t, pl.ds(k1 * 128 + r0, 8), pl.ds(128, 128)])
                         if k1 < (5 if r0 == 0 else 4) else None for k1 in range(8)]
                    res.append(_fft(z, 1))
                for n1 in range(8):
                    for p in range(2):
                        ub[n1, pl.ds(p * 128 + rb * 16, 16), pl.ds(i * 128, 128)] = (
                            jnp.concatenate([res[0][n1][p], res[1][n1][p]], axis=0).astype(BF16))
            yield
        for n1 in range(8):
            yield
            y = _dot(mdi[n1], ub[n1])
            for i in range(CT):
                hf[i, pl.ds(n1, 128, stride=9), :] = y[:, i * 128:(i + 1) * 128]
        return [xs[c * CT + i] + _gather(hf.at[i], D, 8) for i in range(CT)]

    def chain_wo():
        for g in range(4):
            yield from prep_wo(g)

    def middle(first):
        @_loop(0, 3 * NC)
        def _(t):
            g, c = t // NC, t % NC
            _mix((qkv(g + 1, c), 3 * CT), (attn(g, c), 8 * CT))

        if first:
            for c in cps:
                c.wait()
        for c in range(NC + 2):
            _mix(*[(f(*a, c - d), n) for d, (f, a, n) in enumerate((
                (attn, (3,), 8 * CT), (oproj, (), 2 * CT), (fwd, (), 2 * CT + 8)))
                if 0 <= c - d < NC],
                *([(g, 8) for g in [chain_wo()]] if first and c == 0 else []))

        @_loop(0, 32)
        def _(rb):
            r16 = pl.ds(pl.multiple_of(rb * 16, 16), 16)
            for hlf in range(2):
                filt(pl.ds(pl.multiple_of(rb * 16 + hlf * 8, 8), 8),
                     lambda w, k1: w[r16, pl.ds(k1 * 128, 128)].astype(F32)[hlf * 8:hlf * 8 + 8])

        filt(pl.ds(512, 8), lambda w, k1: jnp.broadcast_to(
            w[pl.ds(512, 1), pl.ds(k1 * 128, 128)].astype(F32), (8, 128)))

    def ln0(c):
        for t in range(c * CT, c * CT + CT):
            hb[t] = ln(xs[t]).astype(BF16)
            yield

    _mix((ln0(0), 1))
    for c in range(NC):
        gs = [(qkv(0, c), 3 * CT)]
        if c + 1 < NC:
            gs.append((ln0(c + 1), CT))
        if c == 1:
            for w in wcp[1] + wcp[2] + wcp[3]:
                w.wait()
        if c > 0:
            gs += [(prep_wq(c * 3 + p), 8) for p in range(3)]
        _mix(*gs)
    middle(True)

    def nxt(c):
        for i, x in enumerate((yield from inv(c))):
            xs[c * CT + i] = x
            hb[c * CT + i] = ln(x).astype(BF16)
            yield

    for c in range(NC + 1):
        _mix(*([(nxt(c), 2 * CT + 8)] if c < NC else []),
             *([(qkv(0, c - 1), 3 * CT)] if c else []))
    middle(False)
    def last(c):
        x = yield from inv(c)
        for i in range(0, CT, 2):
            u = (_bits16(x[i]) >> 16) | _bits16(x[i + 1])
            a = (c * CT + i) // 2
            for ct in range(8):
                ut = u[ct * 128:(ct + 1) * 128].T
                for qq in range(4):
                    fin[ct * 4 + qq, pl.ds(a, 32, stride=9), :] = ut[qq * 32:(qq + 1) * 32]
    for c in range(0, NC, 2):
        _mix((last(1 - 1 + c), 12), (last(c + 1), 24))
    for j in range(4):
        for hh in range(2):
            for qq in range(4):
                xio[j, rows(qq), pl.ds(hh * 128, 128)] = pltpu.bitcast(
                    _gather(fin.at[(j * 2 + hh) * 4 + qq], 256, 8), BF16)
        ocp[j].start()
    for c in ocp:
        c.wait()


@jax.jit
def pallas_interleave_layers__sliding_local_dilated__spectral_gfnet__prompt_kernel(
    A_x, A_wqkv, A_wo, B_x, B_w_r, B_w_i,
):
    V = pltpu.VMEM
    L = CT * 128
    scratch = [
        V((4, S, 256), BF16), V((12, D, 256), BF16), V((D, D), BF16),
        V((513, S), BF16), V((513, S), BF16),
        V(_MD.shape, BF16), V(_MDI.shape, BF16), V(_MS.shape, BF16), V(_MSI.shape, BF16),
        V((12, 256, D), BF16), V((D, D), BF16),
        V((NT, D, 128), F32), V((NT, D, 128), BF16),
        V((10 * NT, 128, 128), U32),
        V((32, 288, 128), U32),
        V((NT, D, 128), BF16),
        V((16, R, 256), F32), V((2, CT, R, 256), BF16),
        V((2, CT, 1152, 128), F32), V((2, 8, 256, L), F32), V((2, 8, 256, L), BF16),
        V((3, 8, 272, 128), F32), V((3, 8, 272, 128), F32), V((8, 272, 128), F32), V((2, 1152, 128), U32),
        pltpu.SemaphoreType.DMA((28,)),
    ]
    hbm = pl.BlockSpec(memory_space=pltpu.HBM)
    out = pl.pallas_call(
        _kernel,
        in_specs=[hbm] * 9,
        out_specs=hbm,
        out_shape=jax.ShapeDtypeStruct((S, D), BF16),
        scratch_shapes=scratch,
        compiler_params=pltpu.CompilerParams(vmem_limit_bytes=124 * 1024 * 1024),
    )(A_x.reshape(S, D), A_wqkv, A_wo, B_w_r.T, B_w_i.T, _MD, _MDI, _MS, _MSI)
    return out.reshape(1, S, D)
```

```python
import math

import jax
import jax.numpy as jnp
import numpy as np
import jax.experimental.pallas as pl
import jax.experimental.pallas.tpu as pltpu

S, D = 2048, 1024
NT = S // 128
R = 528
CT = 4
NC = NT // CT
F32, BF16, U32 = jnp.float32, jnp.bfloat16, jnp.uint32


def _consts():
    k2 = np.arange(128)
    md = np.zeros((8, 256, 128), np.float64)
    for n1 in range(8):
        th = 2 * np.pi * ((k2[:, None] * (n1 + 8 * k2[None, :])) % D) / D
        md[n1, :128], md[n1, 128:] = np.cos(th), -np.sin(th)
    ms = np.zeros((16, 256, 256), np.float64)
    for k1 in range(16):
        th = 2 * np.pi * ((k2[None, :] * (k1 + 16 * k2[:, None])) % S) / S
        c, s = np.cos(th), np.sin(th)
        ms[k1] = np.block([[c, -s], [s, c]])
    f = lambda a: np.ascontiguousarray(a).astype(np.float32).astype(BF16)
    return f(md), f(md.transpose(0, 2, 1)), f(ms), f(ms.transpose(0, 2, 1) * (2.0 / (S * D)))


_MD, _MDI, _MS, _MSI = _consts()


def _cadd(a, b):
    if a is None:
        return b
    if b is None:
        return a
    return (a[0] + b[0], a[1] + b[1])


def _bfly(e, o, k, n, sign, want_minus):
    if o is None:
        return e, e
    if k == 0:
        t = o
    elif 4 * k == n:
        if e is None:
            raise NotImplementedError
        p = (e[0] - o[1], e[1] + o[0])
        m = (e[0] + o[1], e[1] - o[0])
        return (p, m) if sign > 0 else (m, p)
    else:
        c, s = math.cos(2 * math.pi * k / n), sign * math.sin(2 * math.pi * k / n)
        if 8 * k == n or 8 * k == 3 * n:
            r = abs(c)
            a, b = o[0] + o[1], o[0] - o[1]
            if c > 0 and s > 0:
                t = (b * r, a * r)
            elif c > 0:
                t = (a * r, b * -r)
            elif s > 0:
                t = (a * -r, b * r)
            else:
                t = (b * -r, a * -r)
        else:
            t = (o[0] * c - o[1] * s, o[0] * s + o[1] * c)
    return _cadd(e, t), ((e[0] - t[0], e[1] - t[1]) if want_minus else None)


def _fft(x, sign, nout=None):
    n = len(x)
    if n == 1:
        return x
    nout = n if nout is None else nout
    e, o = _fft(x[0::2], sign), _fft(x[1::2], sign)
    out = [None] * n
    for k in range(n // 2):
        out[k], out[k + n // 2] = _bfly(e[k], o[k], k, n, sign, k + n // 2 < nout)
    return out[:nout]


def _dot(a, b):
    return jnp.dot(a, b, preferred_element_type=F32)


def _loop(*a, **k):
    def deco(f):
        with jax.named_scope("loop_%d_%d" % a):
            pl.loop(*a, **k)(f)
    return deco


def _spread(ref, v, n):
    for i in range(v.shape[0] // n):
        ref[pl.ds(i * (n + 1), n), :] = v[i * n:(i + 1) * n]


def _gather(ref, rows, n):
    return jnp.concatenate([ref[pl.ds(i * (n + 1), n), :] for i in range(rows // n)], axis=0)


def _unpack(u):
    return (pltpu.bitcast(u << 16, F32), pltpu.bitcast(u & jnp.uint32(0xFFFF0000), F32))


def _mix(*gens):
    ev = sorted(((k + 0.5) / n, i) for i, (_, n) in enumerate(gens) for k in range(n))
    for _, i in ev:
        next(gens[i][0], None)
    for g, _ in gens:
        for _ in g:
            pass


def _bits16(x):
    return pltpu.bitcast(x.astype(BF16).astype(F32), U32)


def _kernel(x_hbm, wqkv_hbm, wo_hbm, wr_hbm, wi_hbm, md_hbm, mdi_hbm, ms_hbm, msi_hbm,
            out_hbm,
            xio, wq_in, wo_in, wr, wi, md, mdi, ms, msi,
            wqt, wot, xs, hb, qkv_s, fin, o_s, cb, ab2, hf2, zb2, ub2, tmp, tmp2, tmp3, xtmp,
            sems):
    srcs = (wo_hbm, md_hbm, ms_hbm, wr_hbm, wi_hbm, msi_hbm, mdi_hbm)
    dsts = (wo_in, md, ms, wr, wi, msi, mdi)
    cps = [pltpu.make_async_copy(s, d, sems.at[i]) for i, (s, d) in enumerate(zip(srcs, dsts))]
    wcp = [[pltpu.make_async_copy(wqkv_hbm.at[:, pl.ds(p * D + g * 256, 256)], wq_in.at[g * 3 + p],
                                  sems.at[8 + g * 3 + p]) for p in range(3)] for g in range(4)]
    cols = lambda r, j: r.at[:, pl.ds(j * 256, 256)]
    xcp = [pltpu.make_async_copy(cols(x_hbm, j), xio.at[j], sems.at[20 + j]) for j in range(4)]
    rows = lambda j: pl.ds(j * 512, 512)
    ocp = [pltpu.make_async_copy(xio.at[j], cols(out_hbm, j), sems.at[24 + j]) for j in range(4)]
    for c in wcp[0] + xcp:
        c.start()

    def ln(x):
        m = jnp.mean(x, axis=0, keepdims=True)
        xc = x - m
        v = jnp.mean(xc * xc, axis=0, keepdims=True)
        return xc * jax.lax.rsqrt(v + 1e-5)

    def prep_wq(gp):
        p = gp % 3
        for ct in range(8):
            tmp[p, ct, pl.ds(0, 256), :] = wq_in[gp, pl.ds(ct * 128, 128), :].astype(F32).T
            for h in range(8):
                for e in range(2):
                    tmp2[p, ct, pl.ds(h * 2 + e, 16, stride=17), :] = (
                        tmp[p, ct, pl.ds(h * 32 + e, 16, stride=2), :])
            wqt[gp, :, pl.ds(ct * 128, 128)] = _gather(tmp2.at[p, ct], 256, 16).astype(BF16)
            yield

    def prep_wo(g):
        for ct in range(8):
            t = tmp3.at[ct]
            _spread(t, wo_in[pl.ds(g * 256, 256), pl.ds(ct * 128, 128)].astype(F32), 32)
            v = jnp.concatenate([t[pl.ds(d, 8, stride=33), :] for d in range(32)], axis=0)
            wot[pl.ds(ct * 128, 128), pl.ds(g * 256, 256)] = v.T.astype(BF16)
            yield

    for c in wcp[0]:
        c.wait()
    _loop(0, 3)(lambda p: _mix((prep_wq(p), 1)))

    for j in range(4):
        xcp[j].wait()
        if j == 3:
            for c in wcp[1] + wcp[2] + wcp[3] + cps:
                c.start()
        for hh in range(2):
            t = xtmp.at[hh]
            _spread(t, pltpu.bitcast(xio[j, :, pl.ds(hh * 128, 128)], U32), 8)
            for a in range(8):
                lo, hi = _unpack(t[pl.ds(a, 128, stride=9), :].T)
                xs[2 * a, pl.ds(j * 256 + hh * 128, 128), :] = lo
                xs[2 * a + 1, pl.ds(j * 256 + hh * 128, 128), :] = hi

    lane0 = jax.lax.broadcasted_iota(jnp.int32, (8, 128), 1) == 0
    lane0_big = jax.lax.broadcasted_iota(jnp.int32, (128, 128), 1) == 0
    row0 = jax.lax.broadcasted_iota(jnp.int32, (8, 128), 0) == 0

    def bufs(g):
        b = (g % 2) * 5 * NT
        return [qkv_s.at[pl.ds(b + o * NT, n * NT)] for o, n in ((0, 1), (1, 2), (3, 2))]

    def qkv(g, c):
        for i in range(CT):
            for p, dst in enumerate(bufs(g)):
                u = pltpu.bitcast(_dot(wqt[g * 3 + p], hb[c * CT + i]).astype(BF16), U32)
                if p == 0:
                    dst[c * CT + i] = u
                else:
                    dst[c * CT + i + NT] = u
                    dst[c * CT + i] = jnp.where(
                        lane0_big, jnp.uint32(0), pltpu.roll(u, 1, 1))
                yield

    def attn(g, c):
        q_s, k_s, v_s = bufs(g)
        for i in range(2):
            t0 = c * CT + i
            lgs = [[None] * 8, [None] * 8]
            for dp in range(16):
                r = pl.ds(dp * 8, 8)
                q = [_unpack(q_s[t0 + 2 * e, r, :]) for e in range(2)]
                for n in range(9):
                    kl, kh = _unpack(k_s[t0 + 2 + NT - 2 * n, r, :])
                    for e in range(2):
                        j = n - 1 + e
                        if 0 <= j < 8:
                            pr = q[e][0] * kl + q[e][1] * kh
                            lgs[e][j] = pr if dp == 0 else lgs[e][j] + pr
                if dp % 2:
                    yield
            a = []
            for e, lg in enumerate(lgs):
                lg = [l * (32 ** -0.5) for l in lg]
                lg = [lg[0]] + [jnp.where(lane0 & (t0 + 2 * e < 2 * j), -1e9, lg[j])
                                for j in range(1, 8)]
                m = lg[0]
                for l in lg[1:]:
                    m = jnp.maximum(m, l)
                ex = [jnp.exp(l - m) for l in lg]
                inv = 1.0 / sum(ex[1:], ex[0])
                a.append([x * inv for x in ex])
            for dp in range(16):
                r = pl.ds(dp * 8, 8)
                o = [None, None]
                for n in range(9):
                    v = _unpack(v_s[t0 + 2 + NT - 2 * n, r, :])
                    for e in range(2):
                        j = n - 1 + e
                        if 0 <= j < 8:
                            o[e] = _cadd(o[e], (a[e][j] * v[0], a[e][j] * v[1]))
                for e in range(2):
                    o_s[t0 + 2 * e, pl.ds(pl.multiple_of(g * 256 + dp * 16, 16), 16), :] = (
                        jnp.concatenate(o[e], axis=0).astype(BF16))
                if dp % 2:
                    yield

    def oproj(c):
        for t in range(c * CT, c * CT + CT):
            for m in range(2):
                r = pl.ds(m * 512, 512)
                xs[t, r, :] += _dot(wot[r, :], o_s[t])
                yield

    def fwd(c):
        hf, zb, ab = hf2.at[c % 2], zb2.at[c % 2], ab2.at[c % 2]
        for i in range(CT):
            _spread(hf.at[i], ln(xs[c * CT + i]), 8)
            yield
        for n1 in range(8):
            rhs = jnp.concatenate(
                [hf[i, pl.ds(n1, 128, stride=9), :].astype(BF16) for i in range(CT)], axis=1)
            zb[n1] = _dot(md[n1], rhs)
            yield
        for i in range(CT):
            for rb in range(8):
                res = []
                for r0 in (rb * 16, rb * 16 + 8):
                    z = [(zb[n1, pl.ds(r0, 8), pl.ds(i * 128, 128)],
                          zb[n1, pl.ds(128 + r0, 8), pl.ds(i * 128, 128)]) for n1 in range(8)]
                    o = _fft(z, -1, 5 if r0 == 0 else 4)
                    if r0 == 0:
                        o[0] = tuple(jnp.where(row0, 0.5 * v, v) for v in o[0])
                        o[4] = tuple(jnp.where(row0, 0.5 * v, 0.0) for v in o[4])
                    elif r0 == 8:
                        o.append((jnp.zeros((8, 128), F32),) * 2)
                    res.append(o)
                for k1 in range(len(res[0])):
                    for p in range(2):
                        ab[i, pl.ds(k1 * 128 + rb * 16, 16), pl.ds(p * 128, 128)] = (
                            jnp.concatenate([res[0][k1][p], res[1][k1][p]], axis=0).astype(BF16))
            cb[c * CT + i] = _dot(ab[i], ms[c * CT + i])
            yield

    def filt(r, w):
        f = _fft([(cb[n, r, pl.ds(0, 128)], cb[n, r, pl.ds(128, 128)]) for n in range(16)], -1)
        g = []
        for k1 in range(16):
            a, b = w(wr, k1), w(wi, k1)
            g.append((f[k1][0] * a - f[k1][1] * b, f[k1][0] * b + f[k1][1] * a))
        for n, v in enumerate(_fft(g, 1)):
            cb[n, r, pl.ds(0, 128)] = v[0]
            cb[n, r, pl.ds(128, 128)] = v[1]

    def inv(c):
        hf, ub = hf2.at[c % 2], ub2.at[c % 2]
        for i in range(CT):
            t = c * CT + i
            cb[t] = _dot(cb[t].astype(BF16), msi[t])
            for rb in range(8):
                res = []
                for r0 in (rb * 16, rb * 16 + 8):
                    z = [(cb[t, pl.ds(k1 * 128 + r0, 8), pl.ds(0, 128)],
                          cb[t, pl.ds(k1 * 128 + r0, 8), pl.ds(128, 128)])
                         if k1 < (5 if r0 == 0 else 4) else None for k1 in range(8)]
                    res.append(_fft(z, 1))
                for n1 in range(8):
                    for p in range(2):
                        ub[n1, pl.ds(p * 128 + rb * 16, 16), pl.ds(i * 128, 128)] = (
                            jnp.concatenate([res[0][n1][p], res[1][n1][p]], axis=0).astype(BF16))
            yield
        for n1 in range(8):
            yield
            y = _dot(mdi[n1], ub[n1])
            for i in range(CT):
                hf[i, pl.ds(n1, 128, stride=9), :] = y[:, i * 128:(i + 1) * 128]
        return [xs[c * CT + i] + _gather(hf.at[i], D, 8) for i in range(CT)]

    def chain_wo():
        for g in range(4):
            yield from prep_wo(g)

    def middle(first):
        @_loop(0, 3 * NC)
        def _(t):
            g, c = t // NC, t % NC
            _mix((qkv(g + 1, c), 3 * CT), (attn(g, c), 8 * CT))

        if first:
            for c in cps:
                c.wait()
        for c in range(NC + 2):
            _mix(*[(f(*a, c - d), n) for d, (f, a, n) in enumerate((
                (attn, (3,), 8 * CT), (oproj, (), 2 * CT), (fwd, (), 2 * CT + 8)))
                if 0 <= c - d < NC],
                *([(g, 8) for g in [chain_wo()]] if first and c == 0 else []))

        @_loop(0, 32)
        def _(rb):
            r16 = pl.ds(pl.multiple_of(rb * 16, 16), 16)
            for hlf in range(2):
                filt(pl.ds(pl.multiple_of(rb * 16 + hlf * 8, 8), 8),
                     lambda w, k1: w[r16, pl.ds(k1 * 128, 128)].astype(F32)[hlf * 8:hlf * 8 + 8])

        filt(pl.ds(512, 8), lambda w, k1: jnp.broadcast_to(
            w[pl.ds(512, 1), pl.ds(k1 * 128, 128)].astype(F32), (8, 128)))

    def ln0(c):
        for t in range(c * CT, c * CT + CT):
            hb[t] = ln(xs[t]).astype(BF16)
            yield

    _mix((ln0(0), 1))
    for c in range(NC):
        gs = [(qkv(0, c), 3 * CT)]
        if c + 1 < NC:
            gs.append((ln0(c + 1), CT))
        if c == 1:
            for w in wcp[1] + wcp[2] + wcp[3]:
                w.wait()
        if c > 0:
            gs += [(prep_wq(c * 3 + p), 8) for p in range(3)]
        _mix(*gs)
    middle(True)

    def nxt(c):
        for i, x in enumerate((yield from inv(c))):
            xs[c * CT + i] = x
            hb[c * CT + i] = ln(x).astype(BF16)
            yield

    for c in range(NC + 1):
        _mix(*([(nxt(c), 2 * CT + 8)] if c < NC else []),
             *([(qkv(0, c - 1), 3 * CT)] if c else []))
    middle(False)
    def last(c):
        x = yield from inv(c)
        for i in range(0, CT, 2):
            u = (_bits16(x[i]) >> 16) | _bits16(x[i + 1])
            a = (c * CT + i) // 2
            for ct in range(8):
                ut = u[ct * 128:(ct + 1) * 128].T
                for qq in range(4):
                    fin[ct * 4 + qq, pl.ds(a, 32, stride=9), :] = ut[qq * 32:(qq + 1) * 32]
    for c in range(0, NC, 2):
        _mix((last(1 - 1 + c), 12), (last(c + 1), 24))
    for j in range(4):
        for hh in range(2):
            for qq in range(4):
                xio[j, rows(qq), pl.ds(hh * 128, 128)] = pltpu.bitcast(
                    _gather(fin.at[(j * 2 + hh) * 4 + qq], 256, 8), BF16)
        ocp[j].start()
    for c in ocp:
        c.wait()


@jax.jit
def pallas_interleave_layers__sliding_local_dilated__spectral_gfnet__prompt_kernel(
    A_x, A_wqkv, A_wo, B_x, B_w_r, B_w_i,
):
    V = pltpu.VMEM
    L = CT * 128
    scratch = [
        V((4, S, 256), BF16), V((12, D, 256), BF16), V((D, D), BF16),
        V((513, S), BF16), V((513, S), BF16),
        V(_MD.shape, BF16), V(_MDI.shape, BF16), V(_MS.shape, BF16), V(_MSI.shape, BF16),
        V((12, 256, D), BF16), V((D, D), BF16),
        V((NT, D, 128), F32), V((NT, D, 128), BF16),
        V((10 * NT, 128, 128), U32),
        V((32, 288, 128), U32),
        V((NT, D, 128), BF16),
        V((16, R, 256), F32), V((2, CT, R, 256), BF16),
        V((2, CT, 1152, 128), F32), V((2, 8, 256, L), F32), V((2, 8, 256, L), BF16),
        V((3, 8, 272, 128), F32), V((3, 8, 272, 128), F32), V((8, 272, 128), F32), V((2, 1152, 128), U32),
        pltpu.SemaphoreType.DMA((28,)),
    ]
    hbm = pl.BlockSpec(memory_space=pltpu.HBM)
    out = pl.pallas_call(
        _kernel,
        in_specs=[hbm] * 9,
        out_specs=hbm,
        out_shape=jax.ShapeDtypeStruct((S, D), BF16),
        scratch_shapes=scratch,
        compiler_params=pltpu.CompilerParams(vmem_limit_bytes=124 * 1024 * 1024),
    )(A_x.reshape(S, D), A_wqkv, A_wo, B_w_r.T, B_w_i.T, _MD, _MDI, _MS, _MSI)
    return out.reshape(1, S, D)
```
